```python
import jax
import jax.numpy as jnp

def _softmax(x, axis=-1):
    return jax.nn.softmax(x, axis=axis)
def _gelu(x):
    return jax.nn.gelu(x, approximate=True)
def _silu(x):
    return jax.nn.silu(x)
def _sigmoid(x):
    return jax.nn.sigmoid(x)
def _layernorm(x, axis=-1, eps=1e-5):
    m = jnp.mean(x, axis=axis, keepdims=True)
    v = jnp.var(x, axis=axis, keepdims=True)
    return (x - m) / jnp.sqrt(v + eps)
def _scatter_add(tgt, idx, src, axis=0):
    return tgt.at[idx].add(src)
def _segment_sum(src, seg, n):
    return jax.ops.segment_sum(src, seg, n)
class _Rng:
    def __init__(self, key):
        self._k = key
    def _next(self):
        self._k, sub = jax.random.split(self._k)
        return sub
    def normal(self, shape):
        return jax.random.normal(self._next(), shape, dtype=jnp.bfloat16)
    def randint(self, lo, hi, shape):
        return jax.random.randint(self._next(), shape, lo, hi, dtype=jnp.int32)
    def uniform(self, shape, lo=0.0, hi=1.0):
        return jax.random.uniform(self._next(), shape, jnp.bfloat16, lo, hi)
    def permutation(self, n):
        return jax.random.permutation(self._next(), n)


kernel_name = 'recurrent_scan__compressed_kv_cla__dense_activation_gelu__decode'

def setup_inputs():
    _rng = _Rng(jax.random.key(int.from_bytes(__import__("os").urandom(4), "little")))
    _w = (lambda a: (lambda t: t.astype(jnp.bfloat16) if jnp.issubdtype(t.dtype, jnp.floating) else t)(jnp.asarray(a)))
    def _A_setup():
        B, H, Sq, Sk, D, M = 2, 32, 1, 16384, 128, 512
        Dc = 4 * D
        return {
            "x": _w((lambda *s: _rng.normal(s) * 0.05)(B, Sq, M)),
            "c_kv": _w((lambda *s: _rng.normal(s) * 0.05)(B, Sk, Dc)),
            "w_q": _w((lambda *s: _rng.normal(s) * 0.05)(M, H, D) * (M ** -0.5)),
            "w_uk": _w((lambda *s: _rng.normal(s) * 0.05)(Dc, H, D) * (Dc ** -0.5)),
            "w_uv": _w((lambda *s: _rng.normal(s) * 0.05)(Dc, H, D) * (Dc ** -0.5)),
            "w_o": _w((lambda *s: _rng.normal(s) * 0.05)(H, D, M) * ((H * D) ** -0.5)),
        }
    _A_in = _A_setup()

    def _B_setup():
        B, S, D, F = 2, 1, 512, 1792
        return {
            "x": _w((lambda *s: _rng.normal(s) * 0.05)(B, S, D)),
            "w1": _w((lambda *s: _rng.normal(s) * 0.05)(D, F) * (D ** -0.5)),
            "b1": _w((lambda *s: _rng.normal(s) * 0.05)(F) * 0.01),
            "w2": _w((lambda *s: _rng.normal(s) * 0.05)(F, D) * (F ** -0.5)),
            "b2": _w((lambda *s: _rng.normal(s) * 0.05)(D) * 0.01),
        }
    _B_in = _B_setup()

    return {
        "A_x": _A_in["x"],
        "A_c_kv": _A_in["c_kv"],
        "A_w_q": _A_in["w_q"],
        "A_w_uk": _A_in["w_uk"],
        "A_w_uv": _A_in["w_uv"],
        "A_w_o": _A_in["w_o"],
        "B_x": _B_in["x"],
        "B_w1": _B_in["w1"],
        "B_b1": _B_in["b1"],
        "B_w2": _B_in["w2"],
        "B_b2": _B_in["b2"],
    }

def reference(A_x, A_c_kv, A_w_q, A_w_uk, A_w_uv, A_w_o, B_x, B_w1, B_b1, B_w2, B_b2):
    def _A_ref(x, c_kv, w_q, w_uk, w_uv, w_o):
        B, Sq, M = x.shape[0], x.shape[1], x.shape[2]
        Sk = c_kv.shape[1]
        H, D = w_q.shape[1], w_q.shape[2]
        q = jnp.einsum("bqm,mhd->bhqd", x, w_q)
        k = jnp.einsum("bkc,chd->bhkd", c_kv, w_uk)
        v = jnp.einsum("bkc,chd->bhkd", c_kv, w_uv)
        scores = jnp.einsum("bhqd,bhkd->bhqk", q, k) * (D ** -0.5)
        off = Sk - Sq
        qi = jnp.arange(Sq)[:, None]
        kj = jnp.arange(Sk)[None, :]
        cmask = kj <= (qi + off)
        scores = jnp.where(cmask[None, None], scores, -1e9)
        p = _softmax(scores, axis=-1)
        ctx = jnp.einsum("bhqk,bhkd->bhqd", p, v)
        return jnp.einsum("bhqd,hdm->bqm", ctx, w_o)

    def _B_ref(x, w1, b1, w2, b2):
        h = jnp.einsum("bsd,df->bsf", x, w1) + b1
        h = _gelu(h)
        return jnp.einsum("bsf,fd->bsd", h, w2) + b2

    x = A_x
    xn = _layernorm(x, axis=-1)
    s = _A_ref(xn, A_c_kv, A_w_q, A_w_uk, A_w_uv, A_w_o)
    g = _silu(_B_ref(xn, B_w1, B_b1, B_w2, B_b2))
    return x + s * g
```

```python
import jax
import jax.numpy as jnp
from jax import lax
import jax.experimental.pallas as pl
import jax.experimental.pallas.tpu as pltpu

F32 = jnp.float32
BF16 = jnp.bfloat16
NT = (((1,), (1,)), ((), ()))

KV_CHUNK = 4096
KV_STEP = 1024
N_SEMS = 3
LANES = 128


def _w2_bounds(F):
    cuts = [c for c in (F - 768, F - 384, F - 128) if c > 0]
    return [0] + cuts + [F]


def _make_kernel(B, M, Sk, Dc, H, D, F):
    NB = B * H
    G = LANES * H
    w2b = _w2_bounds(F)

    def kernel(x_hbm, ckv_hbm, wq_hbm, wuk_hbm, wuv_hbm, wo_hbm, w1_hbm, b1_hbm, w2_hbm, b2_hbm,
               o_ref,
               x_v, ckv_v, wq_v, wuk_v, wuv_v, wo_v, w1_v, b1_v, w2_v, b2_v, e_v, sems):
        groups = []

        def add(*pairs):
            sem = sems.at[len(groups) % N_SEMS]
            groups.append([pltpu.make_async_copy(s, d, sem) for s, d in pairs])
            return len(groups) - 1

        def kick(g):
            if g < len(groups):
                for c in groups[g]:
                    c.start()

        def need(g):
            for c in groups[g]:
                c.wait()
            kick(g + N_SEMS)

        def rows(src, dst, lo, hi):
            return src.at[pl.ds(lo, hi - lo)], dst.at[pl.ds(lo, hi - lo)]

        g_wq = add((wq_hbm, wq_v), (x_hbm, x_v), (b1_hbm, b1_v), (b2_hbm, b2_v))
        g_wuk = add((wuk_hbm, wuk_v))
        g_c = [[add(rows(ckv_hbm.at[b], ckv_v.at[b], i * KV_CHUNK, (i + 1) * KV_CHUNK))
                for i in range(Sk // KV_CHUNK)] for b in range(B)]
        g_w1 = add((w1_hbm, w1_v))
        g_uv = add((wuv_hbm, wuv_v))
        g_wo = add((wo_hbm, wo_v))
        g_w2 = [add(rows(w2_hbm, w2_v, w2b[i], w2b[i + 1])) for i in range(len(w2b) - 1)]
        for g in range(N_SEMS):
            kick(g)

        e_v[...] = (lax.broadcasted_iota(jnp.int32, (LANES, G), 1) // H
                    == lax.broadcasted_iota(jnp.int32, (LANES, G), 0)).astype(BF16)
        hmask = (lax.broadcasted_iota(jnp.int32, (NB, G), 1) % H
                 == lax.broadcasted_iota(jnp.int32, (NB, G), 0) % H)

        def per_head_proj(v, w_v):
            acc = jnp.zeros((NB, D), F32)
            for j in range(v.shape[1] // LANES):
                rep = jnp.dot(v[:, j * LANES:(j + 1) * LANES], e_v[...], preferred_element_type=F32)
                lhs = jnp.where(hmask, rep, 0.0).astype(BF16)
                acc = acc + jnp.dot(lhs, w_v[pl.ds(j * G, G), :], preferred_element_type=F32)
            return acc

        need(g_wq)
        x = x_v[...].astype(F32)
        xc = x - jnp.mean(x, axis=-1, keepdims=True)
        var = jnp.mean(xc * xc, axis=-1, keepdims=True)
        xn = (xc / jnp.sqrt(var + 1e-5)).astype(BF16)
        xr = jnp.concatenate([jnp.broadcast_to(xn[b:b + 1], (H, M)) for b in range(B)], axis=0)
        q = per_head_proj(xr, wq_v)
        qb = (q * (D ** -0.5)).astype(BF16)

        need(g_wuk)
        dmask = (lax.broadcasted_iota(jnp.int32, (LANES, H, NB), 1)
                 == lax.broadcasted_iota(jnp.int32, (LANES, H, NB), 2) % H)
        gsum = (lax.broadcasted_iota(jnp.int32, (LANES, LANES * 8), 1) // 8
                == lax.broadcasted_iota(jnp.int32, (LANES, LANES * 8), 0)).astype(BF16)
        parts = []
        for j in range(Dc // LANES):
            r = lax.dot_general(wuk_v[pl.ds(j * G, G), :], qb, NT, preferred_element_type=F32)
            r = jnp.where(dmask, r.reshape(LANES, H, NB), 0.0)
            r = r.reshape(LANES, H // 8, 8, NB).sum(axis=1)
            r = r.reshape(LANES * 8, NB).astype(BF16)
            parts.append(jnp.dot(gsum, r, preferred_element_type=F32))
        qlat = jnp.concatenate(parts, axis=0).T.astype(BF16)

        ctx = []
        for b in range(B):
            ql = qlat[b * H:(b + 1) * H]
            carry = (jnp.full((H, 1), -jnp.inf, F32), jnp.zeros((H, 1), F32), jnp.zeros((H, Dc), F32))
            for i in range(Sk // KV_CHUNK):
                need(g_c[b][i])

                def step(t, carry, b=b, i=i, ql=ql):
                    m, l, acc = carry
                    k0 = pl.multiple_of(i * KV_CHUNK + t * KV_STEP, KV_STEP)
                    c = ckv_v[b, pl.ds(k0, KV_STEP), :]
                    s = lax.dot_general(ql, c, NT, preferred_element_type=F32)
                    m_new = jnp.maximum(m, jnp.max(s, axis=-1, keepdims=True))
                    alpha = jnp.exp(m - m_new)
                    p = jnp.exp(s - m_new)
                    l = alpha * l + jnp.sum(p, axis=-1, keepdims=True)
                    acc = alpha * acc + jnp.dot(p.astype(BF16), c, preferred_element_type=F32)
                    return m_new, l, acc

                carry = lax.fori_loop(0, KV_CHUNK // KV_STEP, step, carry)
            ctx.append(carry[2] / carry[1])
        ctx_lat = jnp.concatenate(ctx, axis=0).astype(BF16)

        need(g_w1)
        hid = jnp.dot(xn, w1_v[...], preferred_element_type=F32) + b1_v[...].astype(F32)[None, :]
        hid = jax.nn.gelu(hid, approximate=True).astype(BF16)

        need(g_uv)
        cv = per_head_proj(ctx_lat, wuv_v).astype(BF16)

        omask = (lax.broadcasted_iota(jnp.int32, (NB, H * D), 0) % H
                 == lax.broadcasted_iota(jnp.int32, (NB, H * D), 1) // D)
        cvt = jnp.concatenate([cv] * H, axis=1)
        lhs = jnp.where(omask, cvt, jnp.zeros_like(cvt))
        need(g_wo)
        so = jnp.dot(lhs, wo_v[...], preferred_element_type=F32)
        s_out = jnp.sum(so.reshape(B, H, M), axis=1)

        y = jnp.broadcast_to(b2_v[...].astype(F32)[None, :], (B, M))
        for i in range(len(g_w2)):
            need(g_w2[i])
            y = y + jnp.dot(hid[:, w2b[i]:w2b[i + 1]], w2_v[w2b[i]:w2b[i + 1], :],
                            preferred_element_type=F32)
        o_ref[...] = (x + s_out * (y * jax.nn.sigmoid(y))).astype(o_ref.dtype)

    return kernel


@jax.jit
def pallas_recurrent_scan__compressed_kv_cla__dense_activation_gelu__decode_kernel(
    A_x: jax.Array,
    A_c_kv: jax.Array,
    A_w_q: jax.Array,
    A_w_uk: jax.Array,
    A_w_uv: jax.Array,
    A_w_o: jax.Array,
    B_x: jax.Array,
    B_w1: jax.Array,
    B_b1: jax.Array,
    B_w2: jax.Array,
    B_b2: jax.Array,
):
    del B_x
    B, Sq, M = A_x.shape
    _, Sk, Dc = A_c_kv.shape
    _, H, D = A_w_q.shape
    F = B_w1.shape[1]
    assert Sq == 1 and Sk % KV_CHUNK == 0 and KV_CHUNK % KV_STEP == 0
    assert M % LANES == 0 and Dc % LANES == 0 and D == LANES and H % 16 == 0 and F % LANES == 0
    dt = A_x.dtype

    out = pl.pallas_call(
        _make_kernel(B, M, Sk, Dc, H, D, F),
        out_shape=jax.ShapeDtypeStruct((B, M), dt),
        in_specs=[pl.BlockSpec(memory_space=pl.ANY)] * 10,
        out_specs=pl.BlockSpec(memory_space=pltpu.VMEM),
        scratch_shapes=[
            pltpu.VMEM((B, M), dt),
            pltpu.VMEM((B, Sk, Dc), dt),
            pltpu.VMEM((M * H, D), dt),
            pltpu.VMEM((Dc * H, D), dt),
            pltpu.VMEM((Dc * H, D), dt),
            pltpu.VMEM((H * D, M), dt),
            pltpu.VMEM((M, F), dt),
            pltpu.VMEM((F,), dt),
            pltpu.VMEM((F, M), dt),
            pltpu.VMEM((M,), dt),
            pltpu.VMEM((LANES, LANES * H), BF16),
            pltpu.SemaphoreType.DMA((N_SEMS,)),
        ],
        compiler_params=pltpu.CompilerParams(vmem_limit_bytes=100 * 1024 * 1024),
        name="latent_decode_gated",
    )(
        A_x.reshape(B, M),
        A_c_kv,
        A_w_q.reshape(M * H, D),
        A_w_uk.reshape(Dc * H, D),
        A_w_uv.reshape(Dc * H, D),
        A_w_o.reshape(H * D, M),
        B_w1,
        B_b1,
        B_w2,
        B_b2,
    )
    return out.reshape(B, Sq, M)
```
